```python
import jax
import jax.numpy as jnp

def _softmax(x, axis=-1):
    return jax.nn.softmax(x, axis=axis)

def _gelu(x):
    return jax.nn.gelu(x, approximate=True)

def _silu(x):
    return jax.nn.silu(x)

def _sigmoid(x):
    return jax.nn.sigmoid(x)

def _layernorm(x, axis=-1, eps=1e-05):
    m = jnp.mean(x, axis=axis, keepdims=True)
    v = jnp.var(x, axis=axis, keepdims=True)
    return (x - m) / jnp.sqrt(v + eps)

def _scatter_add(tgt, idx, src, axis=0):
    return tgt.at[idx].add(src)

def _segment_sum(src, seg, n):
    return jax.ops.segment_sum(src, seg, n)

class _Rng:

    def __init__(self, key):
        self._k = key

    def _next(self):
        self._k, sub = jax.random.split(self._k)
        return sub

    def normal(self, shape):
        return jax.random.normal(self._next(), shape, dtype=jnp.bfloat16)

    def randint(self, lo, hi, shape):
        return jax.random.randint(self._next(), shape, lo, hi, dtype=jnp.int32)

    def uniform(self, shape, lo=0.0, hi=1.0):
        return jax.random.uniform(self._next(), shape, jnp.bfloat16, lo, hi)

    def permutation(self, n):
        return jax.random.permutation(self._next(), n)
kernel_name = 'adaLN_cond__memory_aug_recurrent_mem_tr__moe_arch_mod__prompt'

def setup_inputs():
    _rng = _Rng(jax.random.key(int.from_bytes(__import__("os").urandom(4), "little")))
    _w = lambda a: (lambda t: t.astype(jnp.bfloat16) if jnp.issubdtype(t.dtype, jnp.floating) else t)(jnp.asarray(a))

    def _A_setup():
        B, S, Dm = (1, 2048, 1024)
        H, Dh = (32, 128)
        M, seg = (8, 32)
        seg = min(seg, S)
        S = S // seg * seg
        return {'x': _w((lambda *s: _rng.normal(s) * 0.05)(B, S, Dm)), 'mem0': _w((lambda *s: _rng.normal(s) * 0.05)(B, M, Dm)), 'Wq': _w((lambda *s: _rng.normal(s) * 0.05)(Dm, H, Dh) * Dm ** (-0.5)), 'Wk': _w((lambda *s: _rng.normal(s) * 0.05)(Dm, H, Dh) * Dm ** (-0.5)), 'Wv': _w((lambda *s: _rng.normal(s) * 0.05)(Dm, H, Dh) * Dm ** (-0.5)), 'Wo': _w((lambda *s: _rng.normal(s) * 0.05)(H, Dh, Dm) * (H * Dh) ** (-0.5)), 'seg_len': seg}
    _A_in = _A_setup()

    def _B_setup():
        B, S, D, F, C = (1, 2048, 1024, 3584, 2)
        return {'x': _w((lambda *s: _rng.normal(s) * 0.05)(B, S, D)), 'w_r': _w((lambda *s: _rng.normal(s) * 0.05)(D)), 'w_gate': _w((lambda *s: _rng.normal(s) * 0.05)(D, F)), 'w_up': _w((lambda *s: _rng.normal(s) * 0.05)(D, F)), 'w_down': _w((lambda *s: _rng.normal(s) * 0.05)(F, D))}
    _B_in = _B_setup()
    return {'A_x': _A_in['x'], 'A_mem0': _A_in['mem0'], 'A_Wq': _A_in['Wq'], 'A_Wk': _A_in['Wk'], 'A_Wv': _A_in['Wv'], 'A_Wo': _A_in['Wo'], 'A_seg_len': _A_in['seg_len'], 'B_x': _B_in['x'], 'B_w_r': _B_in['w_r'], 'B_w_gate': _B_in['w_gate'], 'B_w_up': _B_in['w_up'], 'B_w_down': _B_in['w_down'], 'c': _w((lambda *s: _rng.normal(s) * 0.05)(1, 1024)), 'w_mod': _w((lambda *s: _rng.normal(s) * 0.05)(1024, 6 * 1024) * 1024 ** (-0.5))}

def reference(A_x, A_mem0, A_Wq, A_Wk, A_Wv, A_Wo, A_seg_len, B_x, B_w_r, B_w_gate, B_w_up, B_w_down, c, w_mod):

    def _A_ref(x, mem0, Wq, Wk, Wv, Wo, seg_len):
        B, S, Dm = x.shape
        H, Dh = (Wq.shape[1], Wq.shape[2])
        M = mem0.shape[1]
        scale = Dh ** (-0.5)
        n_seg = S // seg_len
        L = M + seg_len
        idx = jnp.arange(L)
        mask = (idx[:, None] < M) | (idx[:, None] >= idx[None, :])
        mem = mem0
        outs = []
        for s in range(n_seg):
            xs = x[:, s * seg_len:(s + 1) * seg_len, :].copy()
            h = jnp.concatenate([mem, xs], axis=1)
            q = jnp.einsum('btd,dhe->bhte', h, Wq)
            k = jnp.einsum('btd,dhe->bhte', h, Wk)
            v = jnp.einsum('btd,dhe->bhte', h, Wv)
            scores = jnp.einsum('bhqe,bhke->bhqk', q, k) * scale
            scores = jnp.where(mask[None, None], scores, -1000000000.0)
            p = _softmax(scores, axis=-1)
            o = jnp.einsum('bhqk,bhke->bhqe', p, v)
            o = jnp.einsum('bhte,hed->btd', o, Wo)
            mem = o[:, :M, :].copy()
            outs.append(o[:, M:, :])
        return jnp.concatenate(outs, axis=1)

    def _B_ref(x, w_r, w_gate, w_up, w_down):
        B, S, D = x.shape
        C = 2
        r = x @ w_r
        idx = jnp.argsort(-r, axis=-1)[:, :C]
        idx_e = jnp.repeat(idx.reshape(B, C, 1), D, axis=2)
        x_sel = jnp.take_along_axis(x, idx_e, axis=1)
        g = _silu(x_sel @ w_gate)
        u = x_sel @ w_up
        y = g * u @ w_down
        r_sel = _sigmoid(jnp.take_along_axis(r, idx, axis=1))
        y = y * r_sel.reshape(B, C, 1)
        b_off = (jnp.arange(B) * S).reshape(B, 1)
        flat_idx = (idx + b_off).reshape(B * C)
        zero = (x * 0.0).reshape(B * S, D)
        upd = _scatter_add(zero, flat_idx, y.reshape(B * C, D), axis=0)
        return x + upd.reshape(B, S, D)
    x = A_x
    mod = (_silu(c) @ w_mod).reshape(c.shape[0], 6, 1, -1)
    sa, ca, ga, sb, cb, gb = (mod[:, 0].copy(), mod[:, 1].copy(), mod[:, 2].copy(), mod[:, 3].copy(), mod[:, 4].copy(), mod[:, 5].copy())
    h = _layernorm(x, axis=-1) * (1 + ca) + sa
    x = x + ga * _A_ref(h, A_mem0, A_Wq, A_Wk, A_Wv, A_Wo, A_seg_len)
    h = _layernorm(x, axis=-1) * (1 + cb) + sb
    x = x + gb * _B_ref(h, B_w_r, B_w_gate, B_w_up, B_w_down)
    return x
```

```python
import functools

import jax
import jax.numpy as jnp
import numpy as np
from jax import lax
from jax.experimental import pallas as pl
from jax.experimental.pallas import tpu as pltpu

F32 = jnp.float32
BF16 = jnp.bfloat16
U32 = jnp.uint32
EPS = 1e-05
NEG = -1000000000.0


def _ln(x):
    m = jnp.mean(x, axis=-1, keepdims=True)
    d = x - m
    v = jnp.mean(d * d, axis=-1, keepdims=True)
    return d / jnp.sqrt(v + EPS)


def _sigmoid(x):
    return 1.0 / (1.0 + jnp.exp(-x))


def _kernel(c_ref, mem0_ref, wr_ref,
            x_hbm, wq_hbm, wk_hbm, wv_hbm, wo_hbm, wg_hbm, wu_hbm, wd_hbm, wmod_hbm,
            out_hbm,
            W, WO, ring, xb, outb, wmod, wg, wu, wd, hpro, hbuf, obuf, acc, mod, rbuf,
            sem_w, sem_m, sem_o,
            *, S, D, H, M, SEG, XR, R0, RING, G, TAIL):
    NSEG = S // SEG
    L = M + SEG
    scale = 128 ** (-0.5)
    w_hbms = [r.bitcast(U32) for r in (wq_hbm, wk_hbm, wv_hbm)]
    wo32 = wo_hbm.bitcast(U32)

    def w_copy(j, t, p):
        return pltpu.make_async_copy(w_hbms[t].at[:, p, j, :], W.at[(2 * j + p) * 3 + t], sem_w.at[j, t, p])

    cp_moda = pltpu.make_async_copy(wmod_hbm.at[:, 0:2 * D], wmod.at[:, 0:2 * D], sem_m.at[0])
    cp_modb = pltpu.make_async_copy(wmod_hbm.at[:, 2 * D:6 * D], wmod.at[:, 2 * D:6 * D], sem_m.at[1])
    cp_x0 = pltpu.make_async_copy(x_hbm.at[0:R0], xb.at[0:R0], sem_m.at[2])
    cp_x1 = pltpu.make_async_copy(x_hbm.at[R0:S], xb.at[R0:S], sem_m.at[3])
    cp_wo = [pltpu.make_async_copy(wo32.at[:, n * 128:(n + 1) * 128], WO.at[n], sem_m.at[4 + n])
             for n in range(D // 128)]
    nb = 4 + D // 128
    cp_wg = pltpu.make_async_copy(wg_hbm, wg, sem_m.at[nb])
    cp_wu = pltpu.make_async_copy(wu_hbm, wu, sem_m.at[nb + 1])
    cp_wd = pltpu.make_async_copy(wd_hbm, wd, sem_m.at[nb + 2])

    cp_x0.start()
    cp_moda.start()
    for j in range(H // 2):
        for t in range(3):
            for p in range(2):
                w_copy(j, t, p).start()
    for cp in cp_wo:
        cp.start()
    cp_x1.start()
    cp_modb.start()
    cp_wg.start()
    cp_wu.start()
    cp_wd.start()

    def deinterleave(j):
        for t in range(3):
            w_copy(j, t, 0).wait()
            w_copy(j, t, 1).wait()
        for t in range(3):
            ia = (2 * j) * 3 + t
            ib = (2 * j + 1) * 3 + t
            a = W[ia]
            b = W[ib]
            W[ia] = (a & np.uint32(0xFFFF)) | (b << 16)
            W[ib] = (a >> 16) | (b & np.uint32(0xFFFF0000))

    def wtile(i):
        return pltpu.bitcast(W[i], BF16)

    xb[S:S + SEG, :] = jnp.zeros((SEG, D), BF16)
    acc[...] = jnp.zeros((L, D), F32)
    rbuf[...] = jnp.zeros((SEG, 128), F32)
    cc = jnp.broadcast_to(c_ref[...].astype(F32), (8, D))
    sc = (cc * _sigmoid(cc)).astype(BF16)
    cp_moda.wait()
    mod[:, 0:2 * D] = jnp.dot(sc, wmod[:, 0:2 * D], preferred_element_type=F32)
    cp_x0.wait()
    sa = mod[0:1, 0:D]
    ca1 = 1.0 + mod[0:1, D:2 * D]
    PCH = 64
    for i in range(R0 // PCH):
        xr = xb[i * PCH:(i + 1) * PCH, :].astype(F32)
        hpro[i * PCH:(i + 1) * PCH, :] = (_ln(xr) * ca1 + sa).astype(BF16)

    deinterleave(0)

    def pro_body(j, carry):
        @pl.when(j + 1 < H // 2)
        def _():
            deinterleave(j + 1)
        lhs = hpro[...]
        for p in range(2):
            for t in range(3):
                i = (2 * j + p) * 3 + t
                ring[i, 0:R0, :] = jnp.dot(lhs, wtile(i), preferred_element_type=F32)
        return carry

    lax.fori_loop(0, H // 2, pro_body, 0)

    for cp in cp_wo:
        cp.wait()
    cp_x1.wait()
    cp_modb.wait()
    mod[:, 2 * D:6 * D] = jnp.dot(sc, wmod[:, 2 * D:6 * D], preferred_element_type=F32)
    hbuf[0:M, :] = mem0_ref[...].astype(F32)
    hbuf[M:M + XR, :] = _ln(xb[R0:R0 + XR, :].astype(F32)) * ca1 + sa

    row = lax.broadcasted_iota(jnp.int32, (L, 128), 0)
    col = lax.broadcasted_iota(jnp.int32, (L, 128), 1)
    visible = (row < M) | (row >= col)
    fill = jnp.where(col < L, NEG, -jnp.inf).astype(F32)
    keep = visible & (col < L)
    zpad = jnp.zeros((128 - L, 128), F32)
    lane = lax.broadcasted_iota(jnp.int32, (SEG, 128), 1)

    def epilogue(sp):
        r0 = pl.multiple_of(sp * SEG, SEG)
        ga = mod[0:1, 2 * D:3 * D]
        sb = mod[0:1, 3 * D:4 * D]
        cb1 = 1.0 + mod[0:1, 4 * D:5 * D]
        gb = mod[0:1, 5 * D:6 * D]
        x1 = (xb[pl.ds(r0, SEG), :].astype(F32) + ga * acc[M:L, :]).astype(BF16)
        xb[pl.ds(r0, SEG), :] = x1
        x1 = x1.astype(F32)
        h2 = (_ln(x1) * cb1 + sb).astype(BF16).astype(F32)
        r = jnp.sum(h2 * wr_ref[...].astype(F32), axis=-1, keepdims=True)
        rbuf[...] = jnp.where(lane == sp, r, rbuf[...])
        outb[pl.ds(r0, SEG), :] = (x1 + gb * h2).astype(BF16)

    def out_copy(sp):
        r0 = pl.multiple_of(sp * SEG, SEG)
        return pltpu.make_async_copy(outb.at[pl.ds(r0, SEG)], out_hbm.at[pl.ds(r0, SEG)], sem_o.at[0])

    def step(s, carry):
        seg0 = pl.multiple_of(lax.rem(s * SEG, RING), SEG)
        wr_rows = [pl.multiple_of(lax.rem(R0 + s * XR + 8 * i, RING), 8) for i in range(XR // 8)]

        def qkv(h):
            lhs = hbuf[...]
            res = []
            for t in range(3):
                r = jnp.dot(lhs, wtile(3 * h + t), preferred_element_type=F32)
                for i in range(XR // 8):
                    ring[3 * h + t, pl.ds(wr_rows[i], 8), :] = r[M + 8 * i:M + 8 * i + 8, :]
                res.append(r[0:M, :])
            return res

        def full(h, t, m):
            return jnp.concatenate([m, ring[3 * h + t, pl.ds(seg0, SEG), :]], axis=0)

        def scores(h, qm, km):
            kp = jnp.concatenate([full(h, 1, km), zpad], axis=0)
            return lax.dot_general(full(h, 0, qm), kp, (((1,), (1,)), ((), ())), preferred_element_type=F32)

        def softmax(sc_):
            sc_ = jnp.where(keep, sc_ * scale, fill)
            e = jnp.exp(sc_ - jnp.max(sc_, axis=-1, keepdims=True))
            return e, 1.0 / jnp.sum(e, axis=-1, keepdims=True)

        def pv(h, e, rs, vm):
            vp = jnp.concatenate([full(h, 2, vm), zpad], axis=0)
            return jnp.dot(e, vp, preferred_element_type=F32) * rs

        def wo(h0, h1, first):
            lhs = obuf[:, h0 * 128:h1 * 128]
            for n in range(D // 128):
                w = pltpu.bitcast(WO[n, h0 * 64:h1 * 64, :], BF16)
                r = jnp.dot(lhs, w, preferred_element_type=F32)
                if first:
                    acc[:, n * 128:(n + 1) * 128] = r
                else:
                    acc[:, n * 128:(n + 1) * 128] += r

        Q, Sc, P = {}, {}, {}
        done = 0
        for t in range(H + 2):
            if t < H:
                Q[t] = qkv(t)
            else:
                n = min(TAIL, (t - 2) - done)
                if n > 0:
                    wo(done, done + n, done == 0)
                    done += n
            if t == 0:
                epilogue(jnp.where(s == 0, NSEG, s - 1))
            if t == H - 1:
                nxt = pl.multiple_of(jnp.minimum(R0 + (s + 1) * XR, S - XR), 8)
                hbuf[M:M + XR, :] = _ln(xb[pl.ds(nxt, XR), :].astype(F32)) * ca1 + sa
            if 0 <= t - 1 < H:
                Sc[t - 1] = scores(t - 1, Q[t - 1][0], Q[t - 1][1])
            if 0 <= t - 2 < H:
                obuf[:, (t - 2) * 128:(t - 1) * 128] = pv(t - 2, *P[t - 2], Q[t - 2][2])
            if 0 <= t - 1 < H:
                P[t - 1] = softmax(Sc[t - 1])
            if t < H and (t - 3) - done >= G and done + G <= H - 2 * TAIL:
                wo(done, done + G, done == 0)
                done += G
        while done < H:
            n = min(G, H - done)
            wo(done, done + n, done == 0)
            done += n
        hbuf[0:M, :] = acc[0:M, :]

        @pl.when(s > 0)
        def _():
            out_copy(s - 1).start()
        return carry

    lax.fori_loop(0, NSEG, step, 0)
    epilogue(NSEG - 1)
    out_copy(NSEG - 1).start()

    rowi = lax.broadcasted_iota(jnp.int32, (SEG, 128), 0)
    tok = lane * SEG + rowi
    rv = jnp.where(lane < NSEG, rbuf[...], -jnp.inf)
    m1 = jnp.max(rv)
    i1 = jnp.min(jnp.where(rv == m1, tok, S))
    rv2 = jnp.where(tok == i1, -jnp.inf, rv)
    m2 = jnp.max(rv2)
    i2 = jnp.min(jnp.where((rv2 == m2) & (tok != i1), tok, S))
    i1 = jnp.clip(i1, 0, S - 1)
    i2 = jnp.clip(i2, 0, S - 1)

    sub16 = lax.broadcasted_iota(jnp.int32, (16, D), 0)
    sub8 = lax.broadcasted_iota(jnp.int32, (8, D), 0)

    def group(i):
        return pl.multiple_of((i // 16) * 16, 16)

    def pick(buf, i):
        blk = buf[pl.ds(group(i), 16), :].astype(F32)
        return jnp.sum(jnp.where(sub16 == i % 16, blk, 0.0), axis=0, keepdims=True)

    x1s = jnp.where(sub8 == 0, pick(xb, i1), jnp.where(sub8 == 1, pick(xb, i2), 0.0))
    sb = mod[0:1, 3 * D:4 * D]
    cb1 = 1.0 + mod[0:1, 4 * D:5 * D]
    gb = mod[0:1, 5 * D:6 * D]
    h2s = (_ln(x1s) * cb1 + sb).astype(BF16)
    cp_wg.wait()
    cp_wu.wait()
    cp_wd.wait()
    g = jnp.dot(h2s, wg[...], preferred_element_type=F32)
    u = jnp.dot(h2s, wu[...], preferred_element_type=F32)
    a = (g * _sigmoid(g) * u).astype(BF16)
    y = jnp.dot(a, wd[...], preferred_element_type=F32)
    rsel = jnp.where(sub8[:, 0:1] == 0, m1, m2)
    new = x1s + gb * (h2s.astype(F32) + y * _sigmoid(rsel))

    for _ in range(NSEG):
        out_copy(0).wait()

    def patch(i, k):
        g0 = group(i)
        blk = outb[pl.ds(g0, 16), :]
        outb[pl.ds(g0, 16), :] = jnp.where(sub16 == i % 16, new[k:k + 1, :].astype(BF16), blk)

    patch(i1, 0)
    patch(i2, 1)

    def grp_copy(i, k):
        g0 = group(i)
        return pltpu.make_async_copy(outb.at[pl.ds(g0, 16)], out_hbm.at[pl.ds(g0, 16)], sem_o.at[1 + k])

    grp_copy(i1, 0).start()

    @pl.when(group(i1) != group(i2))
    def _():
        grp_copy(i2, 1).start()
        grp_copy(i2, 1).wait()

    grp_copy(i1, 0).wait()


@jax.jit
def pallas_adaLN_cond__memory_aug_recurrent_mem_tr__moe_arch_mod__prompt_kernel(
    A_x, A_mem0, A_Wq, A_Wk, A_Wv, A_Wo, A_seg_len, B_x, B_w_r, B_w_gate, B_w_up, B_w_down, c, w_mod,
):
    del A_seg_len, B_x
    B, S, D = A_x.shape
    H, Dh = A_Wq.shape[1], A_Wq.shape[2]
    M = A_mem0.shape[1]
    F = B_w_gate.shape[1]
    SEG = 32
    assert B == 1 and Dh == 128 and M == 8 and S == 2048 and D == 1024
    XR = SEG - M
    R0 = S - XR * (S // SEG)
    RING = 576
    kern = functools.partial(_kernel, S=S, D=D, H=H, M=M, SEG=SEG, XR=XR, R0=R0, RING=RING, G=4, TAIL=8)
    vmem = pl.BlockSpec(memory_space=pltpu.VMEM)
    hbm = pl.BlockSpec(memory_space=pl.ANY)
    out = pl.pallas_call(
        kern,
        out_shape=jax.ShapeDtypeStruct((S, D), BF16),
        in_specs=[vmem, vmem, vmem] + [hbm] * 9,
        out_specs=hbm,
        scratch_shapes=[
            pltpu.VMEM((3 * H, D // 2, 128), U32),
            pltpu.VMEM((D // 128, H * Dh // 2, 128), U32),
            pltpu.VMEM((3 * H, RING, 128), F32),
            pltpu.VMEM((S + SEG, D), BF16),
            pltpu.VMEM((S + SEG, D), BF16),
            pltpu.VMEM((D, 6 * D), BF16),
            pltpu.VMEM((D, F), BF16),
            pltpu.VMEM((D, F), BF16),
            pltpu.VMEM((F, D), BF16),
            pltpu.VMEM((R0, D), BF16),
            pltpu.VMEM((M + XR, D), F32),
            pltpu.VMEM((M + SEG, H * Dh), F32),
            pltpu.VMEM((M + SEG, D), F32),
            pltpu.VMEM((8, 6 * D), F32),
            pltpu.VMEM((SEG, 128), F32),
            pltpu.SemaphoreType.DMA((H // 2, 3, 2)),
            pltpu.SemaphoreType.DMA((4 + D // 128 + 3,)),
            pltpu.SemaphoreType.DMA((3,)),
        ],
        compiler_params=pltpu.CompilerParams(vmem_limit_bytes=120 * 1024 * 1024),
        name="adaln_rmt_moe",
    )(
        c, A_mem0.reshape(M, D), B_w_r.reshape(1, D),
        A_x.reshape(S, D),
        A_Wq.reshape(D // 2, 2, H, Dh), A_Wk.reshape(D // 2, 2, H, Dh), A_Wv.reshape(D // 2, 2, H, Dh),
        A_Wo.reshape(H * Dh, D), B_w_gate, B_w_up, B_w_down, w_mod,
    )
    return out.reshape(B, S, D)
```

```python
import functools

import jax
import jax.numpy as jnp
import numpy as np
from jax import lax
from jax.experimental import pallas as pl
from jax.experimental.pallas import tpu as pltpu

F32 = jnp.float32
BF16 = jnp.bfloat16
U32 = jnp.uint32
EPS = 1e-05
NEG = -1000000000.0


def _ln(x):
    m = jnp.mean(x, axis=-1, keepdims=True)
    d = x - m
    v = jnp.mean(d * d, axis=-1, keepdims=True)
    return d / jnp.sqrt(v + EPS)


def _sigmoid(x):
    return 1.0 / (1.0 + jnp.exp(-x))


def _kernel(c_ref, mem0_ref, wr_ref,
            x_hbm, wq_hbm, wk_hbm, wv_hbm, wo_hbm, wg_hbm, wu_hbm, wd_hbm, wmod_hbm,
            out_hbm,
            W, WO, ring, xb, outb, wmod, wg, wu, wd, hpro, hbuf, obuf, acc, mod, rbuf,
            sem_w, sem_m, sem_o,
            *, S, D, H, M, SEG, XR, R0, RING, G, TAIL):
    NSEG = S // SEG
    L = M + SEG
    scale = 128 ** (-0.5)
    w_hbms = [r.bitcast(U32) for r in (wq_hbm, wk_hbm, wv_hbm)]
    wo32 = wo_hbm.bitcast(U32)

    def w_copy(j, t, p):
        return pltpu.make_async_copy(w_hbms[t].at[:, p, j, :], W.at[(2 * j + p) * 3 + t], sem_w.at[j, t, p])

    cp_moda = pltpu.make_async_copy(wmod_hbm.at[:, 0:2 * D], wmod.at[:, 0:2 * D], sem_m.at[0])
    cp_modb = pltpu.make_async_copy(wmod_hbm.at[:, 2 * D:6 * D], wmod.at[:, 2 * D:6 * D], sem_m.at[1])
    cp_x0 = pltpu.make_async_copy(x_hbm.at[0:R0], xb.at[0:R0], sem_m.at[2])
    cp_x1 = pltpu.make_async_copy(x_hbm.at[R0:S], xb.at[R0:S], sem_m.at[3])
    cp_wo = [pltpu.make_async_copy(wo32.at[:, n * 128:(n + 1) * 128], WO.at[n], sem_m.at[4 + n])
             for n in range(D // 128)]
    nb = 4 + D // 128
    cp_wg = pltpu.make_async_copy(wg_hbm, wg, sem_m.at[nb])
    cp_wu = pltpu.make_async_copy(wu_hbm, wu, sem_m.at[nb + 1])
    cp_wd = pltpu.make_async_copy(wd_hbm, wd, sem_m.at[nb + 2])

    cp_x0.start()
    cp_moda.start()
    for j in range(H // 2):
        for t in range(3):
            for p in range(2):
                w_copy(j, t, p).start()
    for cp in cp_wo:
        cp.start()
    cp_x1.start()
    cp_modb.start()
    cp_wg.start()
    cp_wu.start()
    cp_wd.start()

    def deinterleave(j):
        for t in range(3):
            w_copy(j, t, 0).wait()
            w_copy(j, t, 1).wait()
        for t in range(3):
            ia = (2 * j) * 3 + t
            ib = (2 * j + 1) * 3 + t
            a = W[ia]
            b = W[ib]
            W[ia] = (a & np.uint32(0xFFFF)) | (b << 16)
            W[ib] = (a >> 16) | (b & np.uint32(0xFFFF0000))

    def wtile(i):
        return pltpu.bitcast(W[i], BF16)

    xb[S:S + SEG, :] = jnp.zeros((SEG, D), BF16)
    acc[...] = jnp.zeros((L, D), F32)
    rbuf[...] = jnp.zeros((SEG, 128), F32)
    cc = jnp.broadcast_to(c_ref[...].astype(F32), (8, D))
    sc = (cc * _sigmoid(cc)).astype(BF16)
    cp_moda.wait()
    mod[:, 0:2 * D] = jnp.dot(sc, wmod[:, 0:2 * D], preferred_element_type=F32)
    cp_x0.wait()
    sa = mod[0:1, 0:D]
    ca1 = 1.0 + mod[0:1, D:2 * D]
    PCH = 64
    for i in range(R0 // PCH):
        xr = xb[i * PCH:(i + 1) * PCH, :].astype(F32)
        hpro[i * PCH:(i + 1) * PCH, :] = (_ln(xr) * ca1 + sa).astype(BF16)

    deinterleave(0)

    def pro_body(j, carry):
        @pl.when(j + 1 < H // 2)
        def _():
            deinterleave(j + 1)
        lhs = hpro[...]
        for p in range(2):
            for t in range(3):
                i = (2 * j + p) * 3 + t
                ring[i, 0:R0, :] = jnp.dot(lhs, wtile(i), preferred_element_type=F32)
        return carry

    lax.fori_loop(0, H // 2, pro_body, 0)

    for cp in cp_wo:
        cp.wait()
    cp_x1.wait()
    cp_modb.wait()
    mod[:, 2 * D:6 * D] = jnp.dot(sc, wmod[:, 2 * D:6 * D], preferred_element_type=F32)
    hbuf[0:M, :] = mem0_ref[...].astype(F32)
    hbuf[M:M + XR, :] = _ln(xb[R0:R0 + XR, :].astype(F32)) * ca1 + sa

    row = lax.broadcasted_iota(jnp.int32, (L, 128), 0)
    col = lax.broadcasted_iota(jnp.int32, (L, 128), 1)
    visible = (row < M) | (row >= col)
    fill = jnp.where(col < L, NEG, -jnp.inf).astype(F32)
    keep = visible & (col < L)
    zpad = jnp.zeros((128 - L, 128), F32)
    lane = lax.broadcasted_iota(jnp.int32, (SEG, 128), 1)

    def epilogue(sp):
        r0 = pl.multiple_of(sp * SEG, SEG)
        ga = mod[0:1, 2 * D:3 * D]
        sb = mod[0:1, 3 * D:4 * D]
        cb1 = 1.0 + mod[0:1, 4 * D:5 * D]
        gb = mod[0:1, 5 * D:6 * D]
        x1 = (xb[pl.ds(r0, SEG), :].astype(F32) + ga * acc[M:L, :]).astype(BF16)
        xb[pl.ds(r0, SEG), :] = x1
        x1 = x1.astype(F32)
        h2 = (_ln(x1) * cb1 + sb).astype(BF16).astype(F32)
        r = jnp.sum(h2 * wr_ref[...].astype(F32), axis=-1, keepdims=True)
        rbuf[...] = jnp.where(lane == sp, r, rbuf[...])
        outb[pl.ds(r0, SEG), :] = (x1 + gb * h2).astype(BF16)

    def out_copy(sp):
        r0 = pl.multiple_of(sp * SEG, SEG)
        return pltpu.make_async_copy(outb.at[pl.ds(r0, SEG)], out_hbm.at[pl.ds(r0, SEG)], sem_o.at[0])

    def step(s, carry):
        seg0 = pl.multiple_of(lax.rem(s * SEG, RING), SEG)
        wr_rows = [pl.multiple_of(lax.rem(R0 + s * XR + 8 * i, RING), 8) for i in range(XR // 8)]

        def qkv(h):
            lhs = hbuf[...]
            return [jnp.dot(lhs, wtile(3 * h + t), preferred_element_type=F32) for t in range(3)]

        def stash(h, res):
            for t in range(3):
                for i in range(XR // 8):
                    ring[3 * h + t, pl.ds(wr_rows[i], 8), :] = res[t][M + 8 * i:M + 8 * i + 8, :]

        def full(h, t, m):
            return jnp.concatenate([m, ring[3 * h + t, pl.ds(seg0, SEG), :]], axis=0)

        def scores(h, qm, km):
            kp = jnp.concatenate([full(h, 1, km), zpad], axis=0)
            return lax.dot_general(full(h, 0, qm), kp, (((1,), (1,)), ((), ())), preferred_element_type=F32)

        def softmax(sc_):
            sc_ = jnp.where(keep, sc_ * scale, fill)
            e = jnp.exp(sc_ - jnp.max(sc_, axis=-1, keepdims=True))
            return e, 1.0 / jnp.sum(e, axis=-1, keepdims=True)

        def pv(h, e, rs, vm):
            vp = jnp.concatenate([full(h, 2, vm), zpad], axis=0)
            return jnp.dot(e, vp, preferred_element_type=F32) * rs

        def wo(h0, h1, first):
            lhs = obuf[:, h0 * 128:h1 * 128]
            for n in range(D // 128):
                w = pltpu.bitcast(WO[n, h0 * 64:h1 * 64, :], BF16)
                r = jnp.dot(lhs, w, preferred_element_type=F32)
                if first:
                    acc[:, n * 128:(n + 1) * 128] = r
                else:
                    acc[:, n * 128:(n + 1) * 128] += r

        Q, Sc, P = {}, {}, {}
        done = 0
        for t in range(H + 2):
            if t < H:
                Q[t] = qkv(t)
            else:
                n = min(TAIL, (t - 2) - done)
                if n > 0:
                    wo(done, done + n, done == 0)
                    done += n
            if t == 0:
                epilogue(jnp.where(s == 0, NSEG, s - 1))
            if t == H - 1:
                nxt = pl.multiple_of(jnp.minimum(R0 + (s + 1) * XR, S - XR), 8)
                hbuf[M:M + XR, :] = _ln(xb[pl.ds(nxt, XR), :].astype(F32)) * ca1 + sa
            if 0 <= t - 1 < H:
                Sc[t - 1] = scores(t - 1, Q[t - 1][0][0:M], Q[t - 1][1][0:M])
            if 0 <= t - 2 < H:
                obuf[:, (t - 2) * 128:(t - 1) * 128] = pv(t - 2, *P[t - 2], Q[t - 2][2][0:M])
            if 0 <= t - 1 < H:
                P[t - 1] = softmax(Sc[t - 1])
            if t < H:
                stash(t, Q[t])
            if t < H and (t - 3) - done >= G and done + G <= H - 2 * TAIL:
                wo(done, done + G, done == 0)
                done += G
        while done < H:
            n = min(G, H - done)
            wo(done, done + n, done == 0)
            done += n
        hbuf[0:M, :] = acc[0:M, :]

        @pl.when(s > 0)
        def _():
            out_copy(s - 1).start()
        return carry

    lax.fori_loop(0, NSEG, step, 0)
    epilogue(NSEG - 1)
    out_copy(NSEG - 1).start()

    rowi = lax.broadcasted_iota(jnp.int32, (SEG, 128), 0)
    tok = lane * SEG + rowi
    rv = jnp.where(lane < NSEG, rbuf[...], -jnp.inf)
    m1 = jnp.max(rv)
    i1 = jnp.min(jnp.where(rv == m1, tok, S))
    rv2 = jnp.where(tok == i1, -jnp.inf, rv)
    m2 = jnp.max(rv2)
    i2 = jnp.min(jnp.where((rv2 == m2) & (tok != i1), tok, S))
    i1 = jnp.clip(i1, 0, S - 1)
    i2 = jnp.clip(i2, 0, S - 1)

    sub16 = lax.broadcasted_iota(jnp.int32, (16, D), 0)
    sub8 = lax.broadcasted_iota(jnp.int32, (8, D), 0)

    def group(i):
        return pl.multiple_of((i // 16) * 16, 16)

    def pick(buf, i):
        blk = buf[pl.ds(group(i), 16), :].astype(F32)
        return jnp.sum(jnp.where(sub16 == i % 16, blk, 0.0), axis=0, keepdims=True)

    x1s = jnp.where(sub8 == 0, pick(xb, i1), jnp.where(sub8 == 1, pick(xb, i2), 0.0))
    sb = mod[0:1, 3 * D:4 * D]
    cb1 = 1.0 + mod[0:1, 4 * D:5 * D]
    gb = mod[0:1, 5 * D:6 * D]
    h2s = (_ln(x1s) * cb1 + sb).astype(BF16)
    cp_wg.wait()
    cp_wu.wait()
    cp_wd.wait()
    g = jnp.dot(h2s, wg[...], preferred_element_type=F32)
    u = jnp.dot(h2s, wu[...], preferred_element_type=F32)
    a = (g * _sigmoid(g) * u).astype(BF16)
    y = jnp.dot(a, wd[...], preferred_element_type=F32)
    rsel = jnp.where(sub8[:, 0:1] == 0, m1, m2)
    new = x1s + gb * (h2s.astype(F32) + y * _sigmoid(rsel))

    for _ in range(NSEG):
        out_copy(0).wait()

    def patch(i, k):
        g0 = group(i)
        blk = outb[pl.ds(g0, 16), :]
        outb[pl.ds(g0, 16), :] = jnp.where(sub16 == i % 16, new[k:k + 1, :].astype(BF16), blk)

    patch(i1, 0)
    patch(i2, 1)

    def grp_copy(i, k):
        g0 = group(i)
        return pltpu.make_async_copy(outb.at[pl.ds(g0, 16)], out_hbm.at[pl.ds(g0, 16)], sem_o.at[1 + k])

    grp_copy(i1, 0).start()

    @pl.when(group(i1) != group(i2))
    def _():
        grp_copy(i2, 1).start()
        grp_copy(i2, 1).wait()

    grp_copy(i1, 0).wait()


@jax.jit
def pallas_adaLN_cond__memory_aug_recurrent_mem_tr__moe_arch_mod__prompt_kernel(
    A_x, A_mem0, A_Wq, A_Wk, A_Wv, A_Wo, A_seg_len, B_x, B_w_r, B_w_gate, B_w_up, B_w_down, c, w_mod,
):
    del A_seg_len, B_x
    B, S, D = A_x.shape
    H, Dh = A_Wq.shape[1], A_Wq.shape[2]
    M = A_mem0.shape[1]
    F = B_w_gate.shape[1]
    SEG = 32
    assert B == 1 and Dh == 128 and M == 8 and S == 2048 and D == 1024
    XR = SEG - M
    R0 = S - XR * (S // SEG)
    RING = 576
    kern = functools.partial(_kernel, S=S, D=D, H=H, M=M, SEG=SEG, XR=XR, R0=R0, RING=RING, G=4, TAIL=8)
    vmem = pl.BlockSpec(memory_space=pltpu.VMEM)
    hbm = pl.BlockSpec(memory_space=pl.ANY)
    out = pl.pallas_call(
        kern,
        out_shape=jax.ShapeDtypeStruct((S, D), BF16),
        in_specs=[vmem, vmem, vmem] + [hbm] * 9,
        out_specs=hbm,
        scratch_shapes=[
            pltpu.VMEM((3 * H, D // 2, 128), U32),
            pltpu.VMEM((D // 128, H * Dh // 2, 128), U32),
            pltpu.VMEM((3 * H, RING, 128), F32),
            pltpu.VMEM((S + SEG, D), BF16),
            pltpu.VMEM((S + SEG, D), BF16),
            pltpu.VMEM((D, 6 * D), BF16),
            pltpu.VMEM((D, F), BF16),
            pltpu.VMEM((D, F), BF16),
            pltpu.VMEM((F, D), BF16),
            pltpu.VMEM((R0, D), BF16),
            pltpu.VMEM((M + XR, D), F32),
            pltpu.VMEM((M + SEG, H * Dh), F32),
            pltpu.VMEM((M + SEG, D), F32),
            pltpu.VMEM((8, 6 * D), F32),
            pltpu.VMEM((SEG, 128), F32),
            pltpu.SemaphoreType.DMA((H // 2, 3, 2)),
            pltpu.SemaphoreType.DMA((4 + D // 128 + 3,)),
            pltpu.SemaphoreType.DMA((3,)),
        ],
        compiler_params=pltpu.CompilerParams(vmem_limit_bytes=120 * 1024 * 1024),
        name="adaln_rmt_moe",
    )(
        c, A_mem0.reshape(M, D), B_w_r.reshape(1, D),
        A_x.reshape(S, D),
        A_Wq.reshape(D // 2, 2, H, Dh), A_Wk.reshape(D // 2, 2, H, Dh), A_Wv.reshape(D // 2, 2, H, Dh),
        A_Wo.reshape(H * Dh, D), B_w_gate, B_w_up, B_w_down, w_mod,
    )
    return out.reshape(B, S, D)
```

```python
import contextlib
import functools

import jax
import jax.numpy as jnp
import numpy as np
from jax import lax
from jax.experimental import pallas as pl
from jax.experimental.pallas import tpu as pltpu

F32 = jnp.float32
BF16 = jnp.bfloat16
U32 = jnp.uint32
EPS = 1e-05
NEG = -1000000000.0
_SCOPES = False
_CFG = dict(G=1, TAIL=7, BFKV=0, EPI_T=2, LN_T=6, LASTG=4)


def _scope(name):
    return jax.named_scope(name) if _SCOPES else contextlib.nullcontext()


def _ln(x):
    m = jnp.mean(x, axis=-1, keepdims=True)
    d = x - m
    v = jnp.mean(d * d, axis=-1, keepdims=True)
    return d / jnp.sqrt(v + EPS)


def _split_lanes(x):
    return jnp.stack([x[:, n * 128:(n + 1) * 128] for n in range(x.shape[1] // 128)], axis=0)


def _sigmoid(x):
    return 1.0 / (1.0 + jnp.exp(-x))


def _kernel(c_ref, mem0_ref, wr_ref,
            x_hbm, wq_hbm, wk_hbm, wv_hbm, wo_hbm, wg_hbm, wu_hbm, wd_hbm, wmod_hbm,
            out_hbm,
            W, WO, ring, xo, wmod, wg, wu, wd, hpro, hbuf, obuf, acc, mod,
            sem_w, sem_m, sem_o,
            *, S, D, H, M, SEG, XR, R0, RING, G, TAIL):
    NSEG = S // SEG
    L = M + SEG
    scale = 128 ** (-0.5)
    w_hbms = [r.bitcast(U32) for r in (wq_hbm, wk_hbm, wv_hbm)]
    wo32 = wo_hbm.bitcast(U32)

    OB = S + SEG

    def w_copy(j, t, p):
        return pltpu.make_async_copy(w_hbms[t].at[:, p, j, :], W.at[(2 * j + p) * 3 + t], sem_w.at[j, t, p])

    NT = D // 128
    NP = H // 2
    mod_cols = [(0, 2 * D)] + [(k * D, (k + 1) * D) for k in range(2, 6)]
    cp_mod = [pltpu.make_async_copy(wmod_hbm.at[:, a:b], wmod.at[:, a:b], sem_m.at[i])
              for i, (a, b) in enumerate(mod_cols)]
    xm = (R0 + S) // 2
    cp_x = [pltpu.make_async_copy(x_hbm.at[a:b], xo.at[a:b], sem_m.at[5 + i])
            for i, (a, b) in enumerate(((0, R0), (R0, xm), (xm, S)))]
    cp_wo = [pltpu.make_async_copy(wo32.at[:, n * 128:(n + 1) * 128], WO.at[n], sem_m.at[8 + n])
             for n in range(NT)]
    cp_b = [pltpu.make_async_copy(src, dst, sem_m.at[8 + NT + i])
            for i, (src, dst) in enumerate(((wg_hbm, wg), (wu_hbm, wu), (wd_hbm, wd)))]

    def start_pair(j):
        for t in range(3):
            for p in range(2):
                w_copy(j, t, p).start()

    AHEAD = 3
    cp_x[0].start()
    cp_mod[0].start()

    def wait_pair(j):
        for t in range(3):
            for p in range(2):
                w_copy(j, t, p).wait()

    def deinterleave(j, t, half):
        rows = pl.ds(half * (D // 4), D // 4)
        ia = (2 * j) * 3 + t
        ib = (2 * j + 1) * 3 + t
        a = W[ia, rows, :]
        b = W[ib, rows, :]
        W[ia, rows, :] = (a & np.uint32(0xFFFF)) | (b << 16)
        W[ib, rows, :] = (a >> 16) | (b & np.uint32(0xFFFF0000))

    def wtile(i):
        return pltpu.bitcast(W[i], BF16)

    xo[S:S + SEG, :] = jnp.zeros((SEG, D), BF16)
    acc[...] = jnp.zeros((L, D), F32)
    ring[3 * H, 0:SEG, :] = jnp.zeros((SEG, 128), F32)
    cc = jnp.broadcast_to(c_ref[...].astype(F32), (8, D))
    sc = (cc * _sigmoid(cc)).astype(BF16)
    PCH = 64
    cp_x[0].wait()
    for i in range(R0 // PCH):
        ring[0:NT, i * PCH:(i + 1) * PCH, :] = _split_lanes(_ln(xo[i * PCH:(i + 1) * PCH, :].astype(F32)))
    cp_mod[0].wait()
    start_pair(0)
    mod[:, 0:2 * D] = jnp.dot(sc, wmod[:, 0:2 * D], preferred_element_type=F32)
    for j in range(1, AHEAD + 1):
        start_pair(j)
    sa = mod[0:1, 0:D]
    ca1 = 1.0 + mod[0:1, D:2 * D]
    for n in range(NT):
        cs = slice(n * 128, (n + 1) * 128)
        hpro[:, cs] = (ring[n, 0:R0, :] * ca1[:, cs] + sa[:, cs]).astype(BF16)

    wait_pair(0)
    for t in range(3):
        for half in range(2):
            deinterleave(0, t, half)

    later = [cp_wo[0:2], cp_wo[2:4], cp_wo[4:6], cp_wo[6:8], cp_x[1:2], cp_x[2:3]] + [[cp] for cp in cp_mod[1:]]

    def pro_body(j, carry):
        @pl.when(j + AHEAD + 1 < NP)
        def _():
            start_pair(j + AHEAD + 1)

        for jj, cps in enumerate(later):
            @pl.when(j == jj)
            def _():
                for cp in cps:
                    cp.start()

        @pl.when(j + 1 < NP)
        def _():
            wait_pair(j + 1)

        for p in range(2):
            for t in range(3):
                i = (2 * j + p) * 3 + t
                ring[i, 0:R0, :] = jnp.dot(hpro[...], wtile(i), preferred_element_type=F32)
        for p in range(2):
            for t in range(3):
                deinterleave(j + 1, t, p)
        return carry

    with _scope('pro_loop'):
        lax.fori_loop(0, NP, pro_body, 0)

    for cp in cp_wo + cp_x[1:] + cp_mod[1:]:
        cp.wait()
    for cp in cp_b:
        cp.start()
    mod[:, 2 * D:6 * D] = jnp.dot(sc, wmod[:, 2 * D:6 * D], preferred_element_type=F32)
    hbuf[0, 0:M, :] = mem0_ref[...].astype(F32)
    hbuf[0, M:M + XR, :] = _ln(xo[R0:R0 + XR, :].astype(F32)) * ca1 + sa

    row = lax.broadcasted_iota(jnp.int32, (L, 128), 0)
    col = lax.broadcasted_iota(jnp.int32, (L, 128), 1)
    visible = (row < M) | (row >= col)
    fill = jnp.where(col < L, NEG, -jnp.inf).astype(F32)
    keep = visible & (col < L)
    zpad = jnp.zeros((128 - L, 128), F32)
    lane = lax.broadcasted_iota(jnp.int32, (SEG, 128), 1)

    def epilogue(sp, rslot):
        r0 = pl.multiple_of(sp * SEG, SEG)
        ga = mod[0:1, 2 * D:3 * D]
        sb = mod[0:1, 3 * D:4 * D]
        cb1 = 1.0 + mod[0:1, 4 * D:5 * D]
        gb = mod[0:1, 5 * D:6 * D]
        x1 = (xo[pl.ds(r0, SEG), :].astype(F32) + ga * acc[M:L, :]).astype(BF16)
        xo[pl.ds(r0, SEG), :] = x1
        x1 = x1.astype(F32)
        h2 = (_ln(x1) * cb1 + sb).astype(BF16).astype(F32)
        r = jnp.sum(h2 * wr_ref[...].astype(F32), axis=-1, keepdims=True)
        ring[rslot, 0:SEG, :] = jnp.where(lane == sp, r, ring[rslot, 0:SEG, :])
        xo[pl.ds(OB + r0, SEG), :] = (x1 + gb * h2).astype(BF16)

    def out_copy(sp):
        r0 = pl.multiple_of(sp * SEG, SEG)
        return pltpu.make_async_copy(xo.at[pl.ds(OB + r0, SEG)], out_hbm.at[pl.ds(r0, SEG)], sem_o.at[0])

    def step(s, carry):
        seg0 = pl.multiple_of(lax.rem(s * SEG, RING), SEG)
        wr_rows = [pl.multiple_of(lax.rem(R0 + s * XR + 8 * i, RING), 8) for i in range(XR // 8)]

        def qkv(h):
            lhs = hbuf[s % 2]
            return [jnp.dot(lhs, wtile(3 * h + t), preferred_element_type=F32) for t in range(3)]

        def stash(h, res):
            for t in range(3):
                for i in range(XR // 8):
                    ring[3 * h + t, pl.ds(wr_rows[i], 8), :] = res[t][M + 8 * i:M + 8 * i + 8, :]

        def full(h, t, m):
            return jnp.concatenate([m, ring[3 * h + t, pl.ds(seg0, SEG), :]], axis=0)

        def scores(h, qm, km):
            kp = jnp.concatenate([full(h, 1, km), zpad], axis=0)
            if _CFG['BFKV']:
                kp = kp.astype(BF16)
            return lax.dot_general(full(h, 0, qm), kp, (((1,), (1,)), ((), ())), preferred_element_type=F32)

        def softmax(sc_):
            sc_ = jnp.where(keep, sc_ * scale, fill)
            e = jnp.exp(sc_ - jnp.max(sc_, axis=-1, keepdims=True))
            return e, 1.0 / jnp.sum(e, axis=-1, keepdims=True)

        def pv(h, e, rs, vm):
            vp = jnp.concatenate([full(h, 2, vm), zpad], axis=0)
            if _CFG['BFKV']:
                vp = vp.astype(BF16)
            return jnp.dot(e, vp, preferred_element_type=F32) * rs

        def wo(h0, h1, first):
            lhs = obuf[:, h0 * 128:h1 * 128]
            for n in range(D // 128):
                w = pltpu.bitcast(WO[n, h0 * 64:h1 * 64, :], BF16)
                r = jnp.dot(lhs, w, preferred_element_type=F32)
                if first:
                    acc[:, n * 128:(n + 1) * 128] = r
                else:
                    acc[:, n * 128:(n + 1) * 128] += r

        Q, Sc, P = {}, {}, {}
        done = 0
        for t in range(H + 2):
            if t < H:
                Q[t] = qkv(t)
            else:
                n = min(TAIL, (t - 2) - done)
                if n > 0:
                    wo(done, done + n, done == 0)
                    done += n
            if t == _CFG['EPI_T']:
                epilogue(jnp.where(s == 0, NSEG, s - 1), 3 * H + s // NSEG)
            if t == _CFG['LN_T']:
                nxt = pl.multiple_of(jnp.minimum(R0 + (s + 1) * XR, S - XR), 8)
                hbuf[(s + 1) % 2, M:M + XR, :] = _ln(xo[pl.ds(nxt, XR), :].astype(F32)) * ca1 + sa
            if 0 <= t - 1 < H:
                Sc[t - 1] = scores(t - 1, Q[t - 1][0][0:M], Q[t - 1][1][0:M])
            if 0 <= t - 2 < H:
                obuf[:, (t - 2) * 128:(t - 1) * 128] = pv(t - 2, *P[t - 2], Q[t - 2][2][0:M])
            if 0 <= t - 1 < H:
                P[t - 1] = softmax(Sc[t - 1])
            if t < H:
                stash(t, Q[t])
            if t < H and (t - 3) - done >= G and done + G <= H - 2 * TAIL:
                wo(done, done + G, done == 0)
                done += G
        while done < H:
            n = min(_CFG['LASTG'], H - done)
            wo(done, done + n, done == 0)
            done += n
        hbuf[(s + 1) % 2, 0:M, :] = acc[0:M, :]

        @pl.when(s > 0)
        def _():
            out_copy(s - 1).start()
        return carry

    with _scope('main_loop'):
        lax.fori_loop(0, NSEG, step, 0)
    epilogue(NSEG - 1, 3 * H)
    out_copy(NSEG - 1).start()

    rowi = lax.broadcasted_iota(jnp.int32, (SEG, 128), 0)
    tok = lane * SEG + rowi
    rv = jnp.where(lane < NSEG, ring[3 * H, 0:SEG, :], -jnp.inf)
    m1 = jnp.max(rv)
    i1 = jnp.min(jnp.where(rv == m1, tok, S))
    rv2 = jnp.where(tok == i1, -jnp.inf, rv)
    m2 = jnp.max(rv2)
    i2 = jnp.min(jnp.where((rv2 == m2) & (tok != i1), tok, S))
    i1 = jnp.clip(i1, 0, S - 1)
    i2 = jnp.clip(i2, 0, S - 1)

    sub16 = lax.broadcasted_iota(jnp.int32, (16, D), 0)
    sub8 = lax.broadcasted_iota(jnp.int32, (8, D), 0)

    def group(i):
        return pl.multiple_of((i // 16) * 16, 16)

    def pick(buf, i):
        blk = buf[pl.ds(group(i), 16), :].astype(F32)
        return jnp.sum(jnp.where(sub16 == i % 16, blk, 0.0), axis=0, keepdims=True)

    x1s = jnp.where(sub8 == 0, pick(xo, i1), jnp.where(sub8 == 1, pick(xo, i2), 0.0))
    sb = mod[0:1, 3 * D:4 * D]
    cb1 = 1.0 + mod[0:1, 4 * D:5 * D]
    gb = mod[0:1, 5 * D:6 * D]
    h2s = (_ln(x1s) * cb1 + sb).astype(BF16)
    for cp in cp_b:
        cp.wait()
    g = jnp.dot(h2s, wg[...], preferred_element_type=F32)
    u = jnp.dot(h2s, wu[...], preferred_element_type=F32)
    a = (g * _sigmoid(g) * u).astype(BF16)
    y = jnp.dot(a, wd[...], preferred_element_type=F32)
    rsel = jnp.where(sub8[:, 0:1] == 0, m1, m2)
    new = x1s + gb * (h2s.astype(F32) + y * _sigmoid(rsel))

    for _ in range(NSEG):
        out_copy(0).wait()

    def patch(i, k):
        g0 = group(i)
        blk = xo[pl.ds(OB + g0, 16), :]
        xo[pl.ds(OB + g0, 16), :] = jnp.where(sub16 == i % 16, new[k:k + 1, :].astype(BF16), blk)

    patch(i1, 0)
    patch(i2, 1)

    def grp_copy(i, k):
        g0 = group(i)
        return pltpu.make_async_copy(xo.at[pl.ds(OB + g0, 16)], out_hbm.at[pl.ds(g0, 16)], sem_o.at[1 + k])

    grp_copy(i1, 0).start()

    @pl.when(group(i1) != group(i2))
    def _():
        grp_copy(i2, 1).start()
        grp_copy(i2, 1).wait()

    grp_copy(i1, 0).wait()


@jax.jit
def pallas_adaLN_cond__memory_aug_recurrent_mem_tr__moe_arch_mod__prompt_kernel(
    A_x, A_mem0, A_Wq, A_Wk, A_Wv, A_Wo, A_seg_len, B_x, B_w_r, B_w_gate, B_w_up, B_w_down, c, w_mod,
):
    del A_seg_len, B_x
    B, S, D = A_x.shape
    H, Dh = A_Wq.shape[1], A_Wq.shape[2]
    M = A_mem0.shape[1]
    F = B_w_gate.shape[1]
    SEG = 32
    assert B == 1 and Dh == 128 and M == 8 and S == 2048 and D == 1024
    XR = SEG - M
    R0 = S - XR * (S // SEG)
    RING = 576
    kern = functools.partial(_kernel, S=S, D=D, H=H, M=M, SEG=SEG, XR=XR, R0=R0, RING=RING, G=_CFG['G'], TAIL=_CFG['TAIL'])
    vmem = pl.BlockSpec(memory_space=pltpu.VMEM)
    hbm = pl.BlockSpec(memory_space=pl.ANY)
    out = pl.pallas_call(
        kern,
        out_shape=jax.ShapeDtypeStruct((S, D), BF16),
        in_specs=[vmem, vmem, vmem] + [hbm] * 9,
        out_specs=hbm,
        scratch_shapes=[
            pltpu.VMEM((3 * H + 6, D // 2, 128), U32),
            pltpu.VMEM((D // 128, H * Dh // 2, 128), U32),
            pltpu.VMEM((3 * H + 1, RING, 128), F32),
            pltpu.VMEM((2 * (S + SEG), D), BF16),
            pltpu.VMEM((D, 6 * D), BF16),
            pltpu.VMEM((D, F), BF16),
            pltpu.VMEM((D, F), BF16),
            pltpu.VMEM((F, D), BF16),
            pltpu.VMEM((R0, D), BF16),
            pltpu.VMEM((2, M + XR, D), F32),
            pltpu.VMEM((M + SEG, H * Dh), F32),
            pltpu.VMEM((M + SEG, D), F32),
            pltpu.VMEM((8, 6 * D), F32),
            pltpu.SemaphoreType.DMA((H // 2, 3, 2)),
            pltpu.SemaphoreType.DMA((8 + D // 128 + 3,)),
            pltpu.SemaphoreType.DMA((3,)),
        ],
        compiler_params=pltpu.CompilerParams(vmem_limit_bytes=120 * 1024 * 1024, disable_bounds_checks=True),
        name="adaln_rmt_moe",
    )(
        c, A_mem0.reshape(M, D), B_w_r.reshape(1, D),
        A_x.reshape(S, D),
        A_Wq.reshape(D // 2, 2, H, Dh), A_Wk.reshape(D // 2, 2, H, Dh), A_Wv.reshape(D // 2, 2, H, Dh),
        A_Wo.reshape(H * Dh, D), B_w_gate, B_w_up, B_w_down, w_mod,
    )
    return out.reshape(B, S, D)
```

```python
import contextlib
import functools

import jax
import jax.numpy as jnp
import numpy as np
from jax import lax
from jax.experimental import pallas as pl
from jax.experimental.pallas import tpu as pltpu

F32 = jnp.float32
BF16 = jnp.bfloat16
U32 = jnp.uint32
EPS = 1e-05
NEG = -1000000000.0
_SCOPES = False
_CFG = dict(G=1, TAIL=(3, 3, 3), LAGW=2, ORDER='qfelspw', BFKV=0, EPI_T=2, LN_T=6, LASTG=4)


def _scope(name):
    return jax.named_scope(name) if _SCOPES else contextlib.nullcontext()


def _ln(x):
    m = jnp.mean(x, axis=-1, keepdims=True)
    d = x - m
    v = jnp.mean(d * d, axis=-1, keepdims=True)
    return d / jnp.sqrt(v + EPS)


def _split_lanes(x):
    return jnp.stack([x[:, n * 128:(n + 1) * 128] for n in range(x.shape[1] // 128)], axis=0)


def _sigmoid(x):
    return 1.0 / (1.0 + jnp.exp(-x))


def _kernel(c_ref, mem0_ref, wr_ref,
            x_hbm, wq_hbm, wk_hbm, wv_hbm, wo_hbm, wg_hbm, wu_hbm, wd_hbm, wmod_hbm,
            out_hbm,
            W, WO, ring, xo, wmod, wg, wu, wd, hpro, hbuf, obuf, acc, ax, mod,
            sem_w, sem_m, sem_o,
            *, S, D, H, M, SEG, XR, R0, RING, G, TAIL):
    NSEG = S // SEG
    L = M + SEG
    scale = 128 ** (-0.5)
    w_hbms = [r.bitcast(U32) for r in (wq_hbm, wk_hbm, wv_hbm)]
    wo32 = wo_hbm.bitcast(U32)

    OB = S + SEG

    def w_copy(j, t, p):
        return pltpu.make_async_copy(w_hbms[t].at[:, p, j, :], W.at[(2 * j + p) * 3 + t], sem_w.at[j, t, p])

    NT = D // 128
    NP = H // 2
    mod_cols = [(0, 2 * D)] + [(k * D // 2, (k + 1) * D // 2) for k in range(4, 12)]
    wmod32 = wmod_hbm.bitcast(U32)
    cp_mod = [pltpu.make_async_copy(wmod32.at[:, a:b], wmod.at[:, a:b], sem_m.at[i])
              for i, (a, b) in enumerate(mod_cols)]
    cp_x = [pltpu.make_async_copy(x_hbm.at[a:b], xo.at[a:b], sem_m.at[9 + i])
            for i, (a, b) in enumerate((k * R0, (k + 1) * R0) for k in range(S // R0))]
    cp_wo = [pltpu.make_async_copy(wo32.at[:, n * 128:(n + 1) * 128], WO.at[n], sem_m.at[13 + n])
             for n in range(NT)]
    cp_b = [pltpu.make_async_copy(src.bitcast(U32), dst, sem_m.at[13 + NT + i])
            for i, (src, dst) in enumerate(((wg_hbm, wg), (wu_hbm, wu), (wd_hbm, wd)))]

    def start_pair(j):
        for t in range(3):
            for p in range(2):
                w_copy(j, t, p).start()

    AHEAD = 3
    cp_x[0].start()
    cp_mod[0].start()
    start_pair(0)

    def wait_pair(j):
        for t in range(3):
            for p in range(2):
                w_copy(j, t, p).wait()

    def deinterleave(j, t, half):
        rows = pl.ds(half * (D // 4), D // 4)
        ia = (2 * j) * 3 + t
        ib = (2 * j + 1) * 3 + t
        a = W[ia, rows, :]
        b = W[ib, rows, :]
        W[ia, rows, :] = (a & np.uint32(0xFFFF)) | (b << 16)
        W[ib, rows, :] = (a >> 16) | (b & np.uint32(0xFFFF0000))

    def wtile(i):
        return pltpu.bitcast(W[i], BF16)

    xo[S:S + SEG, :] = jnp.zeros((SEG, D), BF16)
    ax[...] = jnp.zeros((SEG, D), F32)
    ring[3 * H, 0:SEG, :] = jnp.zeros((SEG, 128), F32)
    cc = jnp.broadcast_to(c_ref[...].astype(F32), (8, D))
    sc = (cc * _sigmoid(cc)).astype(BF16)
    PCH = 64
    with _scope('w_x0'):
        cp_x[0].wait()
    for i in range(R0 // PCH):
        ring[0:NT, i * PCH:(i + 1) * PCH, :] = _split_lanes(_ln(xo[i * PCH:(i + 1) * PCH, :].astype(F32)))
    with _scope('w_mod'):
        cp_mod[0].wait()
    start_pair(1)
    mod[:, 0:2 * D] = jnp.dot(sc, pltpu.bitcast(wmod[:, 0:2 * D], BF16), preferred_element_type=F32)
    sa = mod[0:1, 0:D]
    ca1 = 1.0 + mod[0:1, D:2 * D]
    for n in range(NT):
        cs = slice(n * 128, (n + 1) * 128)
        hpro[:, cs] = (ring[n, 0:R0, :] * ca1[:, cs] + sa[:, cs]).astype(BF16)

    with _scope('w_p0'):
        wait_pair(0)
    start_pair(2)
    for t in range(3):
        for half in range(2):
            deinterleave(0, t, half)

    items = cp_wo + cp_mod[1:] + cp_x[1:]
    later = [items[j * len(items) // (NP - 1):(j + 1) * len(items) // (NP - 1)] for j in range(NP - 1)]

    def pro_body(j, carry, first=False):
        jn = j + 1 + j // NP
        for d in range(6):
            i = 6 * j + d
            ring[i, 0:R0, :] = jnp.dot(hpro[...], wtile(i), preferred_element_type=F32)
            if first:
                if d == 2:
                    wait_pair(1)
                    start_pair(3)
                if d >= 3:
                    deinterleave(1, d - 3, 0)
                    deinterleave(1, d - 3, 1)
            else:
                deinterleave(jn, d // 2, d % 2)

        @pl.when(j + AHEAD + 1 < NP)
        def _():
            start_pair(j + AHEAD + 1)

        for jj, cps in enumerate(later):
            if first == (jj == 0):
                @pl.when(j == jj)
                def _():
                    for cp in cps:
                        cp.start()

        @pl.when(j + 2 < NP)
        def _():
            wait_pair(j + 2)

        return carry

    with _scope('pro_loop'):
        pro_body(jnp.int32(0), 0, first=True)
        lax.fori_loop(1, NP, pro_body, 0)

    with _scope('w_mid'):
        for cp in cp_wo + cp_x[1:] + cp_mod[1:]:
            cp.wait()
    for cp in cp_b:
        cp.start()
    mod[:, 2 * D:6 * D] = jnp.dot(sc, pltpu.bitcast(wmod[:, 2 * D:6 * D], BF16), preferred_element_type=F32)
    hbuf[0, 0:M, :] = mem0_ref[...].astype(F32)
    hbuf[0, M:M + XR, :] = _ln(xo[R0:R0 + XR, :].astype(F32)) * ca1 + sa

    row = lax.broadcasted_iota(jnp.int32, (L, 128), 0)
    col = lax.broadcasted_iota(jnp.int32, (L, 128), 1)
    visible = (row < M) | (row >= col)
    fill = jnp.where(col < L, NEG, -jnp.inf).astype(F32)
    keep = visible & (col < L)
    zpad = jnp.zeros((128 - L, 128), F32)
    lane = lax.broadcasted_iota(jnp.int32, (SEG, 128), 1)

    def epilogue(sp, rslot):
        r0 = pl.multiple_of(sp * SEG, SEG)
        ga = mod[0:1, 2 * D:3 * D]
        sb = mod[0:1, 3 * D:4 * D]
        cb1 = 1.0 + mod[0:1, 4 * D:5 * D]
        gb = mod[0:1, 5 * D:6 * D]
        x1 = (xo[pl.ds(r0, SEG), :].astype(F32) + ga * ax[...]).astype(BF16)
        xo[pl.ds(r0, SEG), :] = x1
        x1 = x1.astype(F32)
        h2 = (_ln(x1) * cb1 + sb).astype(BF16).astype(F32)
        r = jnp.sum(h2 * wr_ref[...].astype(F32), axis=-1, keepdims=True)
        ring[rslot, 0:SEG, :] = jnp.where(lane == sp, r, ring[rslot, 0:SEG, :])
        xo[pl.ds(OB + r0, SEG), :] = (x1 + gb * h2).astype(BF16)

    def out_copy(sp):
        r0 = pl.multiple_of(sp * SEG, SEG)
        return pltpu.make_async_copy(xo.at[pl.ds(OB + r0, SEG)], out_hbm.at[pl.ds(r0, SEG)], sem_o.at[0])

    def step(s, carry):
        seg0 = pl.multiple_of(lax.rem(s * SEG, RING), SEG)
        wr_rows = [pl.multiple_of(lax.rem(R0 + s * XR + 8 * i, RING), 8) for i in range(XR // 8)]

        def qkv(h):
            lhs = hbuf[s % 2]
            return [jnp.dot(lhs, wtile(3 * h + t), preferred_element_type=F32) for t in range(3)]

        def stash(h, res):
            for t in range(3):
                for i in range(XR // 8):
                    ring[3 * h + t, pl.ds(wr_rows[i], 8), :] = res[t][M + 8 * i:M + 8 * i + 8, :]

        def full(h, t, m):
            return jnp.concatenate([m, ring[3 * h + t, pl.ds(seg0, SEG), :]], axis=0)

        def scores(h, qm, km):
            kp = jnp.concatenate([full(h, 1, km), zpad], axis=0)
            if _CFG['BFKV']:
                kp = kp.astype(BF16)
            return lax.dot_general(full(h, 0, qm), kp, (((1,), (1,)), ((), ())), preferred_element_type=F32)

        def softmax(sc_):
            sc_ = jnp.where(keep, sc_ * scale, fill)
            e = jnp.exp(sc_ - jnp.max(sc_, axis=-1, keepdims=True))
            return e, 1.0 / jnp.sum(e, axis=-1, keepdims=True)

        def pv(h, e, rs, vm):
            vp = jnp.concatenate([full(h, 2, vm), zpad], axis=0)
            if _CFG['BFKV']:
                vp = vp.astype(BF16)
            return jnp.dot(e, vp, preferred_element_type=F32) * rs

        def wo(h0, h1, first):
            lhs = obuf[:, h0 * 128:h1 * 128]
            for n in range(D // 128):
                w = pltpu.bitcast(WO[n, h0 * 64:h1 * 64, :], BF16)
                r = jnp.dot(lhs, w, preferred_element_type=F32)
                cs = slice(n * 128, (n + 1) * 128)
                if first:
                    acc[:, cs] = r
                elif h1 < H:
                    acc[:, cs] += r
                else:
                    r = acc[:, cs] + r
                    hbuf[(s + 1) % 2, 0:M, cs] = r[0:M]
                    ax[:, cs] = r[M:L]

        Q, Sc, P = {}, {}, {}
        done = 0
        for t in range(H + 2):
            for op in _CFG['ORDER']:
                if op == 'q' and t < H:
                    Q[t] = qkv(t)
                if op == 'e' and t == _CFG['EPI_T']:
                    epilogue(jnp.where(s == 0, NSEG, s - 1), 3 * H + s // NSEG)
                if op == 'l' and t == _CFG['LN_T']:
                    nxt = pl.multiple_of(jnp.minimum(R0 + (s + 1) * XR, S - XR), 8)
                    hbuf[(s + 1) % 2, M:M + XR, :] = _ln(xo[pl.ds(nxt, XR), :].astype(F32)) * ca1 + sa
                if op == 'f' and t >= H:
                    for _ in range(TAIL[t - H]):
                        wo(done, done + 1, False)
                        done += 1
                if op == 's' and 0 <= t - 1 < H:
                    Sc[t - 1] = scores(t - 1, Q[t - 1][0][0:M], Q[t - 1][1][0:M])
                if op == 'p' and 0 <= t - 2 < H:
                    obuf[:, (t - 2) * 128:(t - 1) * 128] = pv(t - 2, *P[t - 2], Q[t - 2][2][0:M])
                if op == 'w' and t < H and (t - _CFG['LAGW']) - done >= 1 and done + 1 <= H - 1 - sum(TAIL):
                    wo(done, done + 1, done == 0)
                    done += 1
            if 0 <= t - 1 < H:
                P[t - 1] = softmax(Sc[t - 1])
            if t < H:
                stash(t, Q[t])
        while done < H:
            wo(done, done + 1, False)
            done += 1

        @pl.when(s > 0)
        def _():
            out_copy(s - 1).start()
        return carry

    with _scope('main_loop'):
        lax.fori_loop(0, NSEG, step, 0)
    epilogue(NSEG - 1, 3 * H)
    out_copy(NSEG - 1).start()

    rowi = lax.broadcasted_iota(jnp.int32, (SEG, 128), 0)
    tok = lane * SEG + rowi
    rv = jnp.where(lane < NSEG, ring[3 * H, 0:SEG, :], -jnp.inf)
    m1 = jnp.max(rv)
    i1 = jnp.min(jnp.where(rv == m1, tok, S))
    rv2 = jnp.where(tok == i1, -jnp.inf, rv)
    m2 = jnp.max(rv2)
    i2 = jnp.min(jnp.where((rv2 == m2) & (tok != i1), tok, S))
    i1 = jnp.clip(i1, 0, S - 1)
    i2 = jnp.clip(i2, 0, S - 1)

    sub16 = lax.broadcasted_iota(jnp.int32, (16, D), 0)
    sub8 = lax.broadcasted_iota(jnp.int32, (8, D), 0)

    def group(i):
        return pl.multiple_of((i // 16) * 16, 16)

    def pick(buf, i):
        blk = buf[pl.ds(group(i), 16), :].astype(F32)
        return jnp.sum(jnp.where(sub16 == i % 16, blk, 0.0), axis=0, keepdims=True)

    x1s = jnp.where(sub8 == 0, pick(xo, i1), jnp.where(sub8 == 1, pick(xo, i2), 0.0))
    sb = mod[0:1, 3 * D:4 * D]
    cb1 = 1.0 + mod[0:1, 4 * D:5 * D]
    gb = mod[0:1, 5 * D:6 * D]
    h2s = (_ln(x1s) * cb1 + sb).astype(BF16)
    with _scope('w_b'):
        for cp in cp_b:
            cp.wait()
    g = jnp.dot(h2s, pltpu.bitcast(wg[...], BF16), preferred_element_type=F32)
    u = jnp.dot(h2s, pltpu.bitcast(wu[...], BF16), preferred_element_type=F32)
    a = (g * _sigmoid(g) * u).astype(BF16)
    y = jnp.dot(a, pltpu.bitcast(wd[...], BF16), preferred_element_type=F32)
    rsel = jnp.where(sub8[:, 0:1] == 0, m1, m2)
    new = x1s + gb * (h2s.astype(F32) + y * _sigmoid(rsel))

    with _scope('w_out'):
        for _ in range(NSEG):
            out_copy(0).wait()

    def patch(i, k):
        g0 = group(i)
        blk = xo[pl.ds(OB + g0, 16), :]
        xo[pl.ds(OB + g0, 16), :] = jnp.where(sub16 == i % 16, new[k:k + 1, :].astype(BF16), blk)

    patch(i1, 0)
    patch(i2, 1)

    def grp_copy(i, k):
        g0 = group(i)
        return pltpu.make_async_copy(xo.at[pl.ds(OB + g0, 16)], out_hbm.at[pl.ds(g0, 16)], sem_o.at[1 + k])

    grp_copy(i1, 0).start()

    @pl.when(group(i1) != group(i2))
    def _():
        grp_copy(i2, 1).start()
        grp_copy(i2, 1).wait()

    grp_copy(i1, 0).wait()


@jax.jit
def pallas_adaLN_cond__memory_aug_recurrent_mem_tr__moe_arch_mod__prompt_kernel(
    A_x, A_mem0, A_Wq, A_Wk, A_Wv, A_Wo, A_seg_len, B_x, B_w_r, B_w_gate, B_w_up, B_w_down, c, w_mod,
):
    del A_seg_len, B_x
    B, S, D = A_x.shape
    H, Dh = A_Wq.shape[1], A_Wq.shape[2]
    M = A_mem0.shape[1]
    F = B_w_gate.shape[1]
    SEG = 32
    assert B == 1 and Dh == 128 and M == 8 and S == 2048 and D == 1024
    XR = SEG - M
    R0 = S - XR * (S // SEG)
    RING = 576
    kern = functools.partial(_kernel, S=S, D=D, H=H, M=M, SEG=SEG, XR=XR, R0=R0, RING=RING, G=_CFG['G'], TAIL=_CFG['TAIL'])
    vmem = pl.BlockSpec(memory_space=pltpu.VMEM)
    hbm = pl.BlockSpec(memory_space=pl.ANY)
    out = pl.pallas_call(
        kern,
        out_shape=jax.ShapeDtypeStruct((S, D), BF16),
        in_specs=[vmem, vmem, vmem] + [hbm] * 9,
        out_specs=hbm,
        scratch_shapes=[
            pltpu.VMEM((3 * H + 6, D // 2, 128), U32),
            pltpu.VMEM((D // 128, H * Dh // 2, 128), U32),
            pltpu.VMEM((3 * H + 1, RING, 128), F32),
            pltpu.VMEM((2 * (S + SEG), D), BF16),
            pltpu.VMEM((D // 2, 6 * D), U32),
            pltpu.VMEM((D // 2, F), U32),
            pltpu.VMEM((D // 2, F), U32),
            pltpu.VMEM((F // 2, D), U32),
            pltpu.VMEM((R0, D), BF16),
            pltpu.VMEM((2, M + XR, D), F32),
            pltpu.VMEM((M + SEG, H * Dh), F32),
            pltpu.VMEM((M + SEG, D), F32),
            pltpu.VMEM((SEG, D), F32),
            pltpu.VMEM((8, 6 * D), F32),
            pltpu.SemaphoreType.DMA((H // 2, 3, 2)),
            pltpu.SemaphoreType.DMA((13 + D // 128 + 3,)),
            pltpu.SemaphoreType.DMA((3,)),
        ],
        compiler_params=pltpu.CompilerParams(vmem_limit_bytes=120 * 1024 * 1024, disable_bounds_checks=True),
        name="adaln_rmt_moe",
    )(
        c, A_mem0.reshape(M, D), B_w_r.reshape(1, D),
        A_x.reshape(S, D),
        A_Wq.reshape(D // 2, 2, H, Dh), A_Wk.reshape(D // 2, 2, H, Dh), A_Wv.reshape(D // 2, 2, H, Dh),
        A_Wo.reshape(H * Dh, D), B_w_gate, B_w_up, B_w_down, w_mod,
    )
    return out.reshape(B, S, D)
```

```python
import contextlib
import functools

import jax
import jax.numpy as jnp
import numpy as np
from jax import lax
from jax.experimental import pallas as pl
from jax.experimental.pallas import tpu as pltpu

F32 = jnp.float32
BF16 = jnp.bfloat16
U32 = jnp.uint32
EPS = 1e-05
NEG = -1000000000.0
_SCOPES = False
_CFG = dict(G=1, TAIL=(3, 3, 2), LAGW=3, ORDER='qfelswp', BFKV=0, EPI_T=16, LN_T=21, LASTG=4)


def _scope(name):
    return jax.named_scope(name) if _SCOPES else contextlib.nullcontext()


def _ln(x):
    m = jnp.mean(x, axis=-1, keepdims=True)
    d = x - m
    v = jnp.mean(d * d, axis=-1, keepdims=True)
    return d / jnp.sqrt(v + EPS)


def _split_lanes(x):
    return jnp.stack([x[:, n * 128:(n + 1) * 128] for n in range(x.shape[1] // 128)], axis=0)


def _sigmoid(x):
    return 1.0 / (1.0 + jnp.exp(-x))


def _kernel(c_ref, mem0_ref, wr_ref,
            x_hbm, wq_hbm, wk_hbm, wv_hbm, wo_hbm, wg_hbm, wu_hbm, wd_hbm, wmod_hbm,
            out_hbm,
            W, WO, ring, xo, wmod, wg, wu, wd, hpro, hbuf, obuf, acc, ax, mod,
            sem_w, sem_m, sem_o,
            *, S, D, H, M, SEG, XR, R0, RING, G, TAIL):
    NSEG = S // SEG
    L = M + SEG
    scale = 128 ** (-0.5)
    w_hbms = [r.bitcast(U32) for r in (wq_hbm, wk_hbm, wv_hbm)]
    wo32 = wo_hbm.bitcast(U32)

    OB = S + SEG

    def w_copy(j, t, p):
        return pltpu.make_async_copy(w_hbms[t].at[:, p, j, :], W.at[(2 * j + p) * 3 + t], sem_w.at[j, t, p])

    NT = D // 128
    NP = H // 2
    mod_cols = [(0, 2 * D)] + [(k * D // 2, (k + 1) * D // 2) for k in range(4, 12)]
    wmod32 = wmod_hbm.bitcast(U32)
    cp_mod = [pltpu.make_async_copy(wmod32.at[:, a:b], wmod.at[:, a:b], sem_m.at[i])
              for i, (a, b) in enumerate(mod_cols)]
    cp_x = [pltpu.make_async_copy(x_hbm.at[a:b], xo.at[a:b], sem_m.at[9 + i])
            for i, (a, b) in enumerate((k * R0, (k + 1) * R0) for k in range(S // R0))]
    cp_wo = [pltpu.make_async_copy(wo32.at[:, n * 128:(n + 1) * 128], WO.at[n], sem_m.at[13 + n])
             for n in range(NT)]
    cp_b = [pltpu.make_async_copy(src.bitcast(U32), dst, sem_m.at[13 + NT + i])
            for i, (src, dst) in enumerate(((wg_hbm, wg), (wu_hbm, wu), (wd_hbm, wd)))]

    def start_pair(j):
        for t in range(3):
            for p in range(2):
                w_copy(j, t, p).start()

    AHEAD = 3
    cp_x[0].start()
    cp_mod[0].start()
    start_pair(0)

    def wait_pair(j):
        for t in range(3):
            for p in range(2):
                w_copy(j, t, p).wait()

    def deinterleave(j, t, half):
        rows = pl.ds(half * (D // 4), D // 4)
        ia = (2 * j) * 3 + t
        ib = (2 * j + 1) * 3 + t
        a = W[ia, rows, :]
        b = W[ib, rows, :]
        W[ia, rows, :] = (a & np.uint32(0xFFFF)) | (b << 16)
        W[ib, rows, :] = (a >> 16) | (b & np.uint32(0xFFFF0000))

    def wtile(i):
        return pltpu.bitcast(W[i], BF16)

    xo[S:S + SEG, :] = jnp.zeros((SEG, D), BF16)
    ax[...] = jnp.zeros((SEG, D), F32)
    ring[3 * H, 0:SEG, :] = jnp.zeros((SEG, 128), F32)
    cc = jnp.broadcast_to(c_ref[...].astype(F32), (8, D))
    sc = (cc * _sigmoid(cc)).astype(BF16)
    PCH = 64
    with _scope('w_x0'):
        cp_x[0].wait()
    for i in range(R0 // PCH):
        ring[0:NT, i * PCH:(i + 1) * PCH, :] = _split_lanes(_ln(xo[i * PCH:(i + 1) * PCH, :].astype(F32)))
    with _scope('w_mod'):
        cp_mod[0].wait()
    start_pair(1)
    mod[:, 0:2 * D] = jnp.dot(sc, pltpu.bitcast(wmod[:, 0:2 * D], BF16), preferred_element_type=F32)
    sa = mod[0:1, 0:D]
    ca1 = 1.0 + mod[0:1, D:2 * D]
    for n in range(NT):
        cs = slice(n * 128, (n + 1) * 128)
        hpro[:, cs] = (ring[n, 0:R0, :] * ca1[:, cs] + sa[:, cs]).astype(BF16)

    with _scope('w_p0'):
        wait_pair(0)
    start_pair(2)
    for t in range(3):
        for half in range(2):
            deinterleave(0, t, half)

    items = cp_wo + cp_mod[1:] + cp_x[1:]
    later = [items[j * len(items) // (NP - 1):(j + 1) * len(items) // (NP - 1)] for j in range(NP - 1)]

    def pro_body(j, carry, first=False):
        jn = j + 1 + j // NP
        for d in range(6):
            i = 6 * j + d
            ring[i, 0:R0, :] = jnp.dot(hpro[...], wtile(i), preferred_element_type=F32)
            if first:
                if d == 2:
                    wait_pair(1)
                    start_pair(3)
                if d >= 3:
                    deinterleave(1, d - 3, 0)
                    deinterleave(1, d - 3, 1)
            else:
                deinterleave(jn, d // 2, d % 2)

        @pl.when(j + AHEAD + 1 < NP)
        def _():
            start_pair(j + AHEAD + 1)

        for jj, cps in enumerate(later):
            if first == (jj == 0):
                @pl.when(j == jj)
                def _():
                    for cp in cps:
                        cp.start()

        @pl.when(j + 2 < NP)
        def _():
            wait_pair(j + 2)

        return carry

    with _scope('pro_loop'):
        pro_body(jnp.int32(0), 0, first=True)
        lax.fori_loop(1, NP, pro_body, 0)

    with _scope('w_mid'):
        for cp in cp_wo + cp_x[1:] + cp_mod[1:]:
            cp.wait()
    for cp in cp_b:
        cp.start()
    mod[:, 2 * D:6 * D] = jnp.dot(sc, pltpu.bitcast(wmod[:, 2 * D:6 * D], BF16), preferred_element_type=F32)
    hbuf[0, 0:M, :] = mem0_ref[...].astype(F32)
    hbuf[0, M:M + XR, :] = _ln(xo[R0:R0 + XR, :].astype(F32)) * ca1 + sa

    row = lax.broadcasted_iota(jnp.int32, (L, 128), 0)
    col = lax.broadcasted_iota(jnp.int32, (L, 128), 1)
    visible = (row < M) | (row >= col)
    fill = jnp.where(col < L, NEG, -jnp.inf).astype(F32)
    keep = visible & (col < L)
    zpad = jnp.zeros((128 - L, 128), F32)
    lane = lax.broadcasted_iota(jnp.int32, (SEG, 128), 1)

    def epilogue(sp, rslot):
        r0 = pl.multiple_of(sp * SEG, SEG)
        ga = mod[0:1, 2 * D:3 * D]
        sb = mod[0:1, 3 * D:4 * D]
        cb1 = 1.0 + mod[0:1, 4 * D:5 * D]
        gb = mod[0:1, 5 * D:6 * D]
        x1 = (xo[pl.ds(r0, SEG), :].astype(F32) + ga * ax[...]).astype(BF16)
        xo[pl.ds(r0, SEG), :] = x1
        x1 = x1.astype(F32)
        h2 = (_ln(x1) * cb1 + sb).astype(BF16).astype(F32)
        r = jnp.sum(h2 * wr_ref[...].astype(F32), axis=-1, keepdims=True)
        ring[rslot, 0:SEG, :] = jnp.where(lane == sp, r, ring[rslot, 0:SEG, :])
        xo[pl.ds(OB + r0, SEG), :] = (x1 + gb * h2).astype(BF16)

    def out_copy(sp):
        r0 = pl.multiple_of(sp * SEG, SEG)
        return pltpu.make_async_copy(xo.at[pl.ds(OB + r0, SEG)], out_hbm.at[pl.ds(r0, SEG)], sem_o.at[0])

    def step(s, carry):
        seg0 = pl.multiple_of(lax.rem(s * SEG, RING), SEG)
        wr_rows = [pl.multiple_of(lax.rem(R0 + s * XR + 8 * i, RING), 8) for i in range(XR // 8)]

        def qkv(h):
            lhs = hbuf[s % 2]
            return [jnp.dot(lhs, wtile(3 * h + t), preferred_element_type=F32) for t in range(3)]

        def stash(h, res):
            for t in range(3):
                for i in range(XR // 8):
                    ring[3 * h + t, pl.ds(wr_rows[i], 8), :] = res[t][M + 8 * i:M + 8 * i + 8, :]

        def full(h, t, m):
            return jnp.concatenate([m, ring[3 * h + t, pl.ds(seg0, SEG), :]], axis=0)

        def scores(h, qm, km):
            kp = jnp.concatenate([full(h, 1, km), zpad], axis=0)
            if _CFG['BFKV']:
                kp = kp.astype(BF16)
            return lax.dot_general(full(h, 0, qm), kp, (((1,), (1,)), ((), ())), preferred_element_type=F32)

        def softmax(sc_):
            sc_ = jnp.where(keep, sc_ * scale, fill)
            e = jnp.exp(sc_ - jnp.max(sc_, axis=-1, keepdims=True))
            den = jnp.sum(e, axis=-1, keepdims=True)
            r = pl.reciprocal(den, approx=True)
            r = r * (2.0 - den * r)
            return e, r * (2.0 - den * r)

        def pv(h, e, rs, vm):
            vp = jnp.concatenate([full(h, 2, vm), zpad], axis=0)
            if _CFG['BFKV']:
                vp = vp.astype(BF16)
            return jnp.dot(e, vp, preferred_element_type=F32) * rs

        def wo(h0, h1, first):
            lhs = obuf[:, h0 * 128:h1 * 128]
            for n in range(D // 128):
                w = pltpu.bitcast(WO[n, h0 * 64:h1 * 64, :], BF16)
                r = jnp.dot(lhs, w, preferred_element_type=F32)
                cs = slice(n * 128, (n + 1) * 128)
                if first:
                    acc[:, cs] = r
                elif h1 < H:
                    acc[:, cs] += r
                else:
                    r = acc[:, cs] + r
                    hbuf[(s + 1) % 2, 0:M, cs] = r[0:M]
                    ax[:, cs] = r[M:L]

        Q, Sc, P = {}, {}, {}
        done = 0
        for t in range(H + 2):
            for op in _CFG['ORDER']:
                if op == 'q' and t < H:
                    Q[t] = qkv(t)
                if op == 'e' and t == _CFG['EPI_T']:
                    epilogue(jnp.where(s == 0, NSEG, s - 1), 3 * H + s // NSEG)
                if op == 'l' and t == _CFG['LN_T']:
                    nxt = pl.multiple_of(jnp.minimum(R0 + (s + 1) * XR, S - XR), 8)
                    hbuf[(s + 1) % 2, M:M + XR, :] = _ln(xo[pl.ds(nxt, XR), :].astype(F32)) * ca1 + sa
                if op == 'f' and t >= H:
                    for _ in range(TAIL[t - H]):
                        wo(done, done + 1, False)
                        done += 1
                if op == 's' and 0 <= t - 1 < H:
                    Sc[t - 1] = scores(t - 1, Q[t - 1][0][0:M], Q[t - 1][1][0:M])
                if op == 'p' and 0 <= t - 2 < H:
                    obuf[:, (t - 2) * 128:(t - 1) * 128] = pv(t - 2, *P[t - 2], Q[t - 2][2][0:M])
                if op == 'w' and t < H and (t - _CFG['LAGW']) - done >= 1 and done + 1 <= H - 1 - sum(TAIL):
                    wo(done, done + 1, done == 0)
                    done += 1
            if 0 <= t - 1 < H:
                P[t - 1] = softmax(Sc[t - 1])
            if t < H:
                stash(t, Q[t])
        while done < H:
            wo(done, done + 1, False)
            done += 1

        @pl.when(s > 0)
        def _():
            out_copy(s - 1).start()
        return carry

    with _scope('main_loop'):
        lax.fori_loop(0, NSEG, step, 0)
    epilogue(NSEG - 1, 3 * H)
    out_copy(NSEG - 1).start()

    rowi = lax.broadcasted_iota(jnp.int32, (SEG, 128), 0)
    tok = lane * SEG + rowi
    rv = jnp.where(lane < NSEG, ring[3 * H, 0:SEG, :], -jnp.inf)
    m1 = jnp.max(rv)
    i1 = jnp.min(jnp.where(rv == m1, tok, S))
    rv2 = jnp.where(tok == i1, -jnp.inf, rv)
    m2 = jnp.max(rv2)
    i2 = jnp.min(jnp.where((rv2 == m2) & (tok != i1), tok, S))
    i1 = jnp.clip(i1, 0, S - 1)
    i2 = jnp.clip(i2, 0, S - 1)

    sub16 = lax.broadcasted_iota(jnp.int32, (16, D), 0)
    sub8 = lax.broadcasted_iota(jnp.int32, (8, D), 0)

    def group(i):
        return pl.multiple_of((i // 16) * 16, 16)

    def pick(buf, i):
        blk = buf[pl.ds(group(i), 16), :].astype(F32)
        return jnp.sum(jnp.where(sub16 == i % 16, blk, 0.0), axis=0, keepdims=True)

    x1s = jnp.where(sub8 == 0, pick(xo, i1), jnp.where(sub8 == 1, pick(xo, i2), 0.0))
    sb = mod[0:1, 3 * D:4 * D]
    cb1 = 1.0 + mod[0:1, 4 * D:5 * D]
    gb = mod[0:1, 5 * D:6 * D]
    h2s = (_ln(x1s) * cb1 + sb).astype(BF16)
    with _scope('w_b'):
        for cp in cp_b:
            cp.wait()
    g = jnp.dot(h2s, pltpu.bitcast(wg[...], BF16), preferred_element_type=F32)
    u = jnp.dot(h2s, pltpu.bitcast(wu[...], BF16), preferred_element_type=F32)
    a = (g * _sigmoid(g) * u).astype(BF16)
    y = jnp.dot(a, pltpu.bitcast(wd[...], BF16), preferred_element_type=F32)
    rsel = jnp.where(sub8[:, 0:1] == 0, m1, m2)
    new = x1s + gb * (h2s.astype(F32) + y * _sigmoid(rsel))

    with _scope('w_out'):
        for _ in range(NSEG):
            out_copy(0).wait()

    def patch(i, k):
        g0 = group(i)
        blk = xo[pl.ds(OB + g0, 16), :]
        xo[pl.ds(OB + g0, 16), :] = jnp.where(sub16 == i % 16, new[k:k + 1, :].astype(BF16), blk)

    patch(i1, 0)
    patch(i2, 1)

    def grp_copy(i, k):
        g0 = group(i)
        return pltpu.make_async_copy(xo.at[pl.ds(OB + g0, 16)], out_hbm.at[pl.ds(g0, 16)], sem_o.at[1 + k])

    grp_copy(i1, 0).start()

    @pl.when(group(i1) != group(i2))
    def _():
        grp_copy(i2, 1).start()
        grp_copy(i2, 1).wait()

    grp_copy(i1, 0).wait()


@jax.jit
def pallas_adaLN_cond__memory_aug_recurrent_mem_tr__moe_arch_mod__prompt_kernel(
    A_x, A_mem0, A_Wq, A_Wk, A_Wv, A_Wo, A_seg_len, B_x, B_w_r, B_w_gate, B_w_up, B_w_down, c, w_mod,
):
    del A_seg_len, B_x
    B, S, D = A_x.shape
    H, Dh = A_Wq.shape[1], A_Wq.shape[2]
    M = A_mem0.shape[1]
    F = B_w_gate.shape[1]
    SEG = 32
    assert B == 1 and Dh == 128 and M == 8 and S == 2048 and D == 1024
    XR = SEG - M
    R0 = S - XR * (S // SEG)
    RING = 576
    kern = functools.partial(_kernel, S=S, D=D, H=H, M=M, SEG=SEG, XR=XR, R0=R0, RING=RING, G=_CFG['G'], TAIL=_CFG['TAIL'])
    vmem = pl.BlockSpec(memory_space=pltpu.VMEM)
    hbm = pl.BlockSpec(memory_space=pl.ANY)
    out = pl.pallas_call(
        kern,
        out_shape=jax.ShapeDtypeStruct((S, D), BF16),
        in_specs=[vmem, vmem, vmem] + [hbm] * 9,
        out_specs=hbm,
        scratch_shapes=[
            pltpu.VMEM((3 * H + 6, D // 2, 128), U32),
            pltpu.VMEM((D // 128, H * Dh // 2, 128), U32),
            pltpu.VMEM((3 * H + 1, RING, 128), F32),
            pltpu.VMEM((2 * (S + SEG), D), BF16),
            pltpu.VMEM((D // 2, 6 * D), U32),
            pltpu.VMEM((D // 2, F), U32),
            pltpu.VMEM((D // 2, F), U32),
            pltpu.VMEM((F // 2, D), U32),
            pltpu.VMEM((R0, D), BF16),
            pltpu.VMEM((2, M + XR, D), F32),
            pltpu.VMEM((M + SEG, H * Dh), F32),
            pltpu.VMEM((M + SEG, D), F32),
            pltpu.VMEM((SEG, D), F32),
            pltpu.VMEM((8, 6 * D), F32),
            pltpu.SemaphoreType.DMA((H // 2, 3, 2)),
            pltpu.SemaphoreType.DMA((13 + D // 128 + 3,)),
            pltpu.SemaphoreType.DMA((3,)),
        ],
        compiler_params=pltpu.CompilerParams(vmem_limit_bytes=120 * 1024 * 1024, disable_bounds_checks=True),
        name="adaln_rmt_moe",
    )(
        c, A_mem0.reshape(M, D), B_w_r.reshape(1, D),
        A_x.reshape(S, D),
        A_Wq.reshape(D // 2, 2, H, Dh), A_Wk.reshape(D // 2, 2, H, Dh), A_Wv.reshape(D // 2, 2, H, Dh),
        A_Wo.reshape(H * Dh, D), B_w_gate, B_w_up, B_w_down, w_mod,
    )
    return out.reshape(B, S, D)
```
